```python
import jax
import jax.numpy as jnp

def _softmax(x, axis=-1):
    return jax.nn.softmax(x, axis=axis)
def _gelu(x):
    return jax.nn.gelu(x, approximate=True)
def _silu(x):
    return jax.nn.silu(x)
def _sigmoid(x):
    return jax.nn.sigmoid(x)
def _layernorm(x, axis=-1, eps=1e-5):
    m = jnp.mean(x, axis=axis, keepdims=True)
    v = jnp.var(x, axis=axis, keepdims=True)
    return (x - m) / jnp.sqrt(v + eps)
def _scatter_add(tgt, idx, src, axis=0):
    return tgt.at[idx].add(src)
def _segment_sum(src, seg, n):
    return jax.ops.segment_sum(src, seg, n)
class _Rng:
    def __init__(self, key):
        self._k = key
    def _next(self):
        self._k, sub = jax.random.split(self._k)
        return sub
    def normal(self, shape):
        return jax.random.normal(self._next(), shape, dtype=jnp.bfloat16)
    def randint(self, lo, hi, shape):
        return jax.random.randint(self._next(), shape, lo, hi, dtype=jnp.int32)
    def uniform(self, shape, lo=0.0, hi=1.0):
        return jax.random.uniform(self._next(), shape, jnp.bfloat16, lo, hi)
    def permutation(self, n):
        return jax.random.permutation(self._next(), n)


kernel_name = 'standalone__depthwise_separable__vision'

def setup_inputs():
    _rng = _Rng(jax.random.key(int.from_bytes(__import__("os").urandom(4), "little")))
    _w = (lambda a: (lambda t: t.astype(jnp.bfloat16) if jnp.issubdtype(t.dtype, jnp.floating) else t)(jnp.asarray(a)))
    H = W = 384
    C = 384
    k = 1
    return {
        "x": _w((lambda *s: _rng.normal(s) * 0.05)(1, H, W, C)),
        "dw": _w((lambda *s: _rng.normal(s) * 0.05)(k, k, C)),
        "pw": _w((lambda *s: _rng.normal(s) * 0.05)(C, C)),
    }

def reference(x, dw, pw):
    B, H, W, C = x.shape
    k = dw.shape[0]
    pad = k // 2
    xp = jnp.pad(x, ((0,0),(pad,pad),(pad,pad),(0,0)))
    out = jnp.zeros_like(x)
    for i in range(k):
        for j in range(k):
            out = out + xp[:, i:i+H, j:j+W, :] * dw[i, j][None, None, None, :]
    return jnp.einsum('bhwc,cd->bhwd', out, pw)
```

```python
import jax
import jax.numpy as jnp
import jax.experimental.pallas as pl
import jax.experimental.pallas.tpu as pltpu


def _kernel(x_ref, dw_ref, pw_ref, o_ref):
    t = (x_ref[...].astype(jnp.float32) * dw_ref[0].astype(jnp.float32)).astype(jnp.bfloat16)
    o_ref[...] = jnp.dot(t, pw_ref[...], preferred_element_type=jnp.float32).astype(o_ref.dtype)


@jax.jit
def pallas_standalone__depthwise_separable__vision_kernel(x, dw, pw):
    B, H, W, C = x.shape
    D = pw.shape[1]
    M = B * H * W
    tm = 2048
    out = pl.pallas_call(
        _kernel,
        grid=(M // tm,),
        in_specs=[
            pl.BlockSpec((tm, C), lambda i: (i, 0)),
            pl.BlockSpec((1, 1, C), lambda i: (0, 0, 0)),
            pl.BlockSpec((C, D), lambda i: (0, 0)),
        ],
        out_specs=pl.BlockSpec((tm, D), lambda i: (i, 0)),
        out_shape=jax.ShapeDtypeStruct((M, D), x.dtype),
        compiler_params=pltpu.CompilerParams(
            dimension_semantics=("parallel",), vmem_limit_bytes=100 * 1024 * 1024),
    )(x.reshape(M, C), dw, pw)
    return out.reshape(B, H, W, D)
```

```python
import functools

import jax
import jax.numpy as jnp
from jax import lax
import jax.experimental.pallas as pl
import jax.experimental.pallas.tpu as pltpu

_TILE = 512
_WRITE_ROWS = 3072
_READ_EIGHTHS = (1, 2, 5)


def _kernel(x_hbm, dw_hbm, pw_hbm, o_hbm, buf, dw_v, pw_v, rsem, psem, wsem,
            *, bounds):
    n_stages = len(bounds) - 1
    m = bounds[-1]
    switch = bounds[-2]

    def read(s):
        rows = pl.ds(bounds[s], bounds[s + 1] - bounds[s])
        return pltpu.make_async_copy(x_hbm.at[rows], buf.at[rows], rsem.at[s])

    def write(start, size):
        rows = pl.ds(start, size)
        return pltpu.make_async_copy(buf.at[rows], o_hbm.at[rows], wsem.at[0])

    def compute(start, size):
        def tile(i, carry):
            rows = pl.ds(pl.multiple_of(start + i * _TILE, _TILE), _TILE)
            scale = dw_v[0].astype(jnp.float32)
            t = (buf[rows, :].astype(jnp.float32) * scale).astype(buf.dtype)
            y = jnp.dot(t, pw_v[...], preferred_element_type=jnp.float32)
            buf[rows, :] = y.astype(buf.dtype)
            return carry

        lax.fori_loop(0, size // _TILE, tile, 0)

    read(0).start()
    dw_copy = pltpu.make_async_copy(dw_hbm, dw_v, psem.at[0])
    pw_copy = pltpu.make_async_copy(pw_hbm, pw_v, psem.at[1])
    dw_copy.start()
    pw_copy.start()
    read(1).start()
    dw_copy.wait()
    pw_copy.wait()

    for s in range(n_stages - 1):
        read(s).wait()
        if s + 2 < n_stages:
            read(s + 2).start()
        compute(bounds[s], bounds[s + 1] - bounds[s])
    read(n_stages - 1).wait()

    write(0, switch).start()

    def step(j, carry):
        start = pl.multiple_of(switch + j * _WRITE_ROWS, _TILE)
        compute(start, _WRITE_ROWS)
        write(start, _WRITE_ROWS).start()
        return carry

    lax.fori_loop(0, (m - switch) // _WRITE_ROWS, step, 0)
    pltpu.make_async_copy(buf, o_hbm, wsem.at[0]).wait()


@jax.jit
def pallas_standalone__depthwise_separable__vision_kernel(x, dw, pw):
    b, h, w, c = x.shape
    m = b * h * w
    assert dw.shape == (1, 1, c) and pw.shape == (c, c)
    bounds = [0]
    for eighths in _READ_EIGHTHS:
        bounds.append(bounds[-1] + eighths * (m // 8))
    assert bounds[-1] == m and (m // 8) % _TILE == 0
    assert (m - bounds[-2]) % _WRITE_ROWS == 0 and _WRITE_ROWS % _TILE == 0

    out = pl.pallas_call(
        functools.partial(_kernel, bounds=tuple(bounds)),
        in_specs=[pl.BlockSpec(memory_space=pl.ANY)] * 3,
        out_specs=pl.BlockSpec(memory_space=pl.ANY),
        out_shape=jax.ShapeDtypeStruct((m, c), x.dtype),
        scratch_shapes=[
            pltpu.VMEM((m, c), x.dtype),
            pltpu.VMEM(dw.shape, dw.dtype),
            pltpu.VMEM(pw.shape, pw.dtype),
            pltpu.SemaphoreType.DMA((len(_READ_EIGHTHS),)),
            pltpu.SemaphoreType.DMA((2,)),
            pltpu.SemaphoreType.DMA((1,)),
        ],
        compiler_params=pltpu.CompilerParams(
            vmem_limit_bytes=120 * 1024 * 1024),
    )(x.reshape(m, c), dw, pw)
    return out.reshape(b, h, w, c)
```

```python
import functools

import jax
import jax.numpy as jnp
from jax import lax
import jax.experimental.pallas as pl
import jax.experimental.pallas.tpu as pltpu

_STREAMS = 6
_PIECE = 48
_TILE = 2
_PRIME = 4


def _kernel(x_hbm, dw_hbm, pw_hbm, o_hbm, buf, dw_v, pw_v, rsem, psem, wsem,
            *, stages):
    streams, _, c = buf.shape
    n_stages = len(stages) - 1
    rounds = stages[-1]
    half = stages[-2]

    def read(s):
        rows = pl.ds(stages[s] * _PIECE, (stages[s + 1] - stages[s]) * _PIECE)
        return pltpu.make_async_copy(
            x_hbm.at[:, rows], buf.at[:, rows], rsem.at[s])

    def write(j):
        rows = pl.ds(pl.multiple_of(j * _PIECE, _PIECE), _PIECE)
        return pltpu.make_async_copy(
            buf.at[:, rows], o_hbm.at[:, rows], wsem.at[0])

    def compute(j):
        rows = pl.ds(pl.multiple_of(j * _PIECE, _PIECE), _TILE * _PIECE)
        x = buf[:, rows, :].reshape(streams * _TILE * _PIECE, c)
        t = x.astype(jnp.float32) * dw_v[0].astype(jnp.float32)
        y = jnp.dot(t.astype(buf.dtype), pw_v[...],
                    preferred_element_type=jnp.float32)
        buf[:, rows, :] = y.astype(buf.dtype).reshape(
            streams, _TILE * _PIECE, c)

    dw_copy = pltpu.make_async_copy(dw_hbm, dw_v, psem.at[0])
    pw_copy = pltpu.make_async_copy(pw_hbm, pw_v, psem.at[1])
    dw_copy.start()
    pw_copy.start()
    read(0).start()
    dw_copy.wait()
    pw_copy.wait()
    for s in range(1, n_stages):
        read(s).start()

    for s in range(n_stages - 1):
        read(s).wait()

        @pl.loop(0, (stages[s + 1] - stages[s]) // _TILE)
        def _(i, first=stages[s]):
            compute(first + i * _TILE)

    read(n_stages - 1).wait()

    for j in range(_PRIME):
        write(j).start()

    @pl.loop(0, (rounds - half) // _TILE)
    def _(i):
        compute(half + i * _TILE)
        done = half + (i + 1) * _TILE
        lo = jnp.minimum(_PRIME + i * 2 * _TILE, done - _TILE)
        hi = jnp.minimum(_PRIME + (i + 1) * 2 * _TILE, done)
        for k in range(2 * _TILE):
            @pl.when(lo + k < hi)
            def _():
                write(lo + k).start()

    pltpu.make_async_copy(buf, o_hbm, wsem.at[0]).wait()


@jax.jit
def pallas_standalone__depthwise_separable__vision_kernel(x, dw, pw):
    b, h, w, c = x.shape
    m = b * h * w
    assert dw.shape == (1, 1, c) and pw.shape == (c, c)
    assert m % (_STREAMS * _PIECE * _TILE * 32) == 0
    rows = m // _STREAMS
    rounds = rows // _PIECE
    stages = (0, rounds // 32, rounds // 8, rounds // 4, rounds // 2, rounds)

    out = pl.pallas_call(
        functools.partial(_kernel, stages=stages),
        in_specs=[pl.BlockSpec(memory_space=pl.ANY)] * 3,
        out_specs=pl.BlockSpec(memory_space=pl.ANY),
        out_shape=jax.ShapeDtypeStruct((_STREAMS, rows, c), x.dtype),
        scratch_shapes=[
            pltpu.VMEM((_STREAMS, rows, c), x.dtype),
            pltpu.VMEM(dw.shape, dw.dtype),
            pltpu.VMEM(pw.shape, pw.dtype),
            pltpu.SemaphoreType.DMA((len(stages) - 1,)),
            pltpu.SemaphoreType.DMA((2,)),
            pltpu.SemaphoreType.DMA((1,)),
        ],
        compiler_params=pltpu.CompilerParams(
            vmem_limit_bytes=120 * 1024 * 1024),
    )(x.reshape(_STREAMS, rows, c), dw, pw)
    return out.reshape(b, h, w, c)
```

```python
import jax
import jax.numpy as jnp
import jax.experimental.pallas as pl
import jax.experimental.pallas.tpu as pltpu

_STREAMS = 6
_PIECE = 48
_TILE = 4
_PRIME = 16
_TAIL = 32


def _kernel(x_hbm, dw_hbm, pw_hbm, o_hbm, buf, dw_v, pw_v, wsem):
    streams, rows, c = buf.shape
    rounds = rows // _PIECE
    early = (rounds + _PRIME) // 2
    stages = [0, rounds // 32, rounds // 8, rounds // 4, early]
    bounds = [s * _PIECE for s in stages] + [rows - _TAIL, rows]
    n_reads = len(bounds) - 1

    def write(j):
        sl = pl.ds(pl.multiple_of(j * _PIECE, _PIECE), _PIECE)
        return pltpu.make_async_copy(buf.at[:, sl], o_hbm.at[:, sl], wsem.at[0])

    def compute(j):
        sl = pl.ds(pl.multiple_of(j * _PIECE, _PIECE), _TILE * _PIECE)
        x = buf[:, sl, :].reshape(streams * _TILE * _PIECE, c)
        t = x.astype(jnp.float32) * dw_v[0].astype(jnp.float32)
        y = jnp.dot(t.astype(buf.dtype), pw_v[...],
                    preferred_element_type=jnp.float32)
        buf[:, sl, :] = y.astype(buf.dtype).reshape(streams, _TILE * _PIECE, c)

    def read_phase(rsem):
        def read(s):
            sl = pl.ds(bounds[s], bounds[s + 1] - bounds[s])
            return pltpu.make_async_copy(
                x_hbm.at[:, sl], buf.at[:, sl], rsem.at[s])

        dw_copy = pltpu.make_async_copy(dw_hbm, dw_v, rsem.at[n_reads])
        pw_copy = pltpu.make_async_copy(pw_hbm, pw_v, rsem.at[n_reads + 1])
        dw_copy.start()
        pw_copy.start()
        read(0).start()
        dw_copy.wait()
        pw_copy.wait()
        for s in range(1, n_reads):
            read(s).start()

        for s in range(len(stages) - 1):
            read(s).wait()

            @pl.loop(0, (stages[s + 1] - stages[s]) // _TILE)
            def _(i, first=stages[s]):
                compute(first + i * _TILE)

        read(n_reads - 2).wait()
        for j in range(_PRIME):
            write(j).start()
        read(n_reads - 1).wait()

    pl.run_scoped(read_phase, pltpu.SemaphoreType.DMA((n_reads + 2,)))

    @pl.loop(0, (rounds - early) // _TILE)
    def _(i):
        compute(early + i * _TILE)
        for k in range(2 * _TILE):
            write(_PRIME + i * 2 * _TILE + k).start()

    pltpu.make_async_copy(buf, o_hbm, wsem.at[0]).wait()


@jax.jit
def pallas_standalone__depthwise_separable__vision_kernel(x, dw, pw):
    b, h, w, c = x.shape
    m = b * h * w
    assert dw.shape == (1, 1, c) and pw.shape == (c, c)
    assert m % (_STREAMS * _PIECE * _TILE * 32) == 0
    assert _PRIME % (2 * _TILE) == 0
    rows = m // _STREAMS

    out = pl.pallas_call(
        _kernel,
        in_specs=[pl.BlockSpec(memory_space=pl.ANY)] * 3,
        out_specs=pl.BlockSpec(memory_space=pl.ANY),
        out_shape=jax.ShapeDtypeStruct((_STREAMS, rows, c), x.dtype),
        scratch_shapes=[
            pltpu.VMEM((_STREAMS, rows, c), x.dtype),
            pltpu.VMEM(dw.shape, dw.dtype),
            pltpu.VMEM(pw.shape, pw.dtype),
            pltpu.SemaphoreType.DMA((1,)),
        ],
        compiler_params=pltpu.CompilerParams(
            vmem_limit_bytes=120 * 1024 * 1024),
    )(x.reshape(_STREAMS, rows, c), dw, pw)
    return out.reshape(b, h, w, c)
```
